```python
import os as _os
_os.environ.setdefault("JAX_PLATFORMS", "cpu")
import jax
import jax.numpy as jnp

def _softmax(x, axis=-1):
    return jax.nn.softmax(x, axis=axis)
def _gelu(x):
    return jax.nn.gelu(x, approximate=True)
def _silu(x):
    return jax.nn.silu(x)
def _sigmoid(x):
    return jax.nn.sigmoid(x)
def _layernorm(x, axis=-1, eps=1e-5):
    m = jnp.mean(x, axis=axis, keepdims=True)
    v = jnp.var(x, axis=axis, keepdims=True)
    return (x - m) / jnp.sqrt(v + eps)
def _scatter_add(tgt, idx, src, axis=0):
    return tgt.at[idx].add(src)
def _segment_sum(src, seg, n):
    return jax.ops.segment_sum(src, seg, n)
class _Rng:
    def __init__(self, key):
        self._k = key
    def _next(self):
        self._k, sub = jax.random.split(self._k)
        return sub
    def normal(self, shape):
        return jax.random.normal(self._next(), shape, dtype=jnp.bfloat16)
    def randint(self, lo, hi, shape):
        return jax.random.randint(self._next(), shape, lo, hi, dtype=jnp.int32)
    def uniform(self, shape, lo=0.0, hi=1.0):
        return jax.random.uniform(self._next(), shape, jnp.bfloat16, lo, hi)
    def permutation(self, n):
        return jax.random.permutation(self._next(), n)


kernel_name = 'standalone__mha_block_cached__near_ridge'

def setup_inputs():
    _rng = _Rng(jax.random.key(int.from_bytes(__import__("os").urandom(4), "little")))
    _w = (lambda a: (lambda t: t.astype(jnp.bfloat16) if jnp.issubdtype(t.dtype, jnp.floating) else t)(jnp.asarray(a)))
    B, Sq, D = 8, 96, 576
    H, Sk, Dh = 32, 96, 128
    return {
        "x": _w((lambda *s: _rng.normal(s) * 0.8)(B, Sq, D)),
        "k_cache": _w((lambda *s: _rng.normal(s) * 0.8)(B, H, Sk, Dh)),
        "v_cache": _w((lambda *s: _rng.normal(s) * 0.05)(B, H, Sk, Dh)),
        "wq": _w((lambda *s: _rng.normal(s) * 0.8)(D, H * Dh) * (D ** -0.5)),
        "wo": _w((lambda *s: _rng.normal(s) * 0.05)(H * Dh, D) * ((H * Dh) ** -0.5)),
    }

def reference(x, k_cache, v_cache, wq, wo):
    B, Sq, D = x.shape
    H, Dh = 32, 128
    q = (lambda x, *d: x.transpose(*d))((x @ wq).reshape(B, Sq, H, Dh), 0, 2, 1, 3)
    scores = jnp.einsum("bhqd,bhkd->bhqk", q, k_cache) * (Dh ** -0.5)
    p = _softmax(scores, axis=-1)
    o = jnp.einsum("bhqk,bhkd->bhqd", p, v_cache)
    return (lambda x, *d: x.transpose(*d))(o, 0, 2, 1, 3).reshape(B, Sq, H * Dh) @ wo
```

```python
import jax, jax.numpy as jnp, math
from jax import lax
import jax.experimental.pallas as pl
import jax.experimental.pallas.tpu as pltpu

B, SQ, D, H, SK, DH = 8, 96, 576, 32, 96, 128
NT = (((1,), (1,)), ((), ()))
G = 4
NG = H // G
GW = G * DH
KR = G * SK
BF = jnp.bfloat16
F32 = jnp.float32

def mo(v, n):
    return v if isinstance(v, int) else pl.multiple_of(v, n)

@jax.jit
def pallas_standalone__mha_block_cached__near_ridge_kernel(x, k_cache, v_cache, wq, wo):
    approx, order, osched, QL = True, "SQPO", (5, -1, 0, 1, 2, -1, 3, 4), 3
    c = (DH ** -0.5) * math.log2(math.e)

    def kern(x_hbm, k_hbm, v_hbm, wq_hbm, wo_hbm, out_hbm,
             x_s, k_s, v_s, wq_s, wo_s, q_s, p_s, l_s, o_s, acc, out_s, sem, osem):
        def cp_x(i):
            r = pl.ds(i * 192, 192)
            return pltpu.make_async_copy(x_hbm.at[r], x_s.at[r], sem.at[4, i])
        def cp_o(t):
            r = pl.ds(t * 128, 128)
            return pltpu.make_async_copy(out_s.at[r], out_hbm.at[r], osem.at[t])
        def cp_wq(g):
            return pltpu.make_async_copy(wq_hbm.at[:, pl.ds(mo(g * GW, GW), GW)], wq_s.at[g], sem.at[0, g])
        def cp_wo(g):
            return pltpu.make_async_copy(wo_hbm.at[:, pl.ds(mo(g * GW, GW), GW)], wo_s.at[g], sem.at[1, g])
        def cp_k(g):
            return pltpu.make_async_copy(k_hbm.at[:, pl.ds(mo(g * KR, KR), KR), :], k_s.at[g, :, pl.ds(0, KR), :], sem.at[2, g])
        def cp_v(g):
            return pltpu.make_async_copy(v_hbm.at[:, pl.ds(mo(g * KR, KR), KR), :], v_s.at[g, :, pl.ds(0, KR), :], sem.at[3, g])

        cp_wq(0).start(); cp_x(0).start()
        cp_x(1).start(); cp_k(0).start()
        acc[...] = jnp.zeros_like(acc)
        for g in range(NG):
            v_s[g, :, KR:KR + 32, :] = jnp.zeros((B, 32, DH), BF)
        lane = lax.broadcasted_iota(jnp.int32, (SQ, 128), 1)

        def Q(g, b):
            q = jnp.dot(x_s[b * SQ:(b + 1) * SQ, :], wq_s[g], preferred_element_type=F32)
            q_s[b % 4] = (q * c).astype(BF)
        def S(g, b):
            for h in range(G):
                s = lax.dot_general(q_s[b % 4, :, h * DH:(h + 1) * DH], k_s[g, b, h * SK:h * SK + 128, :], NT, preferred_element_type=F32)
                s = jnp.where(lane < SK, s, -jnp.inf)
                m = jnp.max(s, axis=1, keepdims=True)
                p = jnp.exp2(s - m)
                l = jnp.sum(p, axis=1, keepdims=True)
                p_s[b % 2, h] = p.astype(BF)
                l_s[b % 2, h] = jnp.broadcast_to(pl.reciprocal(l, approx=approx), (SQ, 128))
        def P(g, b):
            for h in range(G):
                o = jnp.dot(p_s[b % 2, h], v_s[g, b, h * SK:h * SK + 128, :], preferred_element_type=F32)
                o_s[b * SQ:(b + 1) * SQ, h * DH:(h + 1) * DH] = (o * l_s[b % 2, h]).astype(BF)
        def O(g, t, fin=False):
            r = lax.dot_general(wo_s[g], o_s[t * 128:(t + 1) * 128, :], NT, preferred_element_type=F32)
            if fin:
                out_s[t * 128:(t + 1) * 128, :] = (acc[:, t * 128:(t + 1) * 128] + r).T.astype(BF)
                cp_o(t).start()
            else:
                acc[:, t * 128:(t + 1) * 128] += r

        cp_wq(0).wait(); cp_x(0).wait()
        cp_x(2).start(); cp_x(3).start(); cp_v(0).start(); cp_wo(0).start()
        Q(0, 0); Q(0, 1)
        cp_x(1).wait(); cp_k(0).wait()
        cp_wq(1).start(); cp_k(1).start(); cp_v(1).start(); cp_wo(1).start()
        if QL == 3: Q(0, 2)
        S(0, 0)
        cp_x(2).wait(); cp_x(3).wait(); cp_v(0).wait(); cp_wo(0).wait()

        def fin(t):
            out_s[t * 128:(t + 1) * 128, :] = acc[:, t * 128:(t + 1) * 128].T.astype(BF)
            cp_o(t).start()

        def slot(g, b, first=False, last=False):
            for op in order:
                if op == "Q":
                    if b + QL < B: Q(g, b + QL)
                    elif not last: Q(g + 1, b + QL - B)
                elif op == "S":
                    if b + 1 < B: S(g, b + 1)
                    elif not last: S(g + 1, 0)
                elif op == "P":
                    P(g, b)
                elif op == "O":
                    t = osched[b]
                    if t == 5:
                        if not first: O(g - 1, 5)
                    elif t >= 0:
                        O(g, t, last)
        R = B - QL
        for b in range(R):
            slot(0, b, first=True)

        def loop_body(g, _):
            @pl.when(g + 2 < NG)
            def _():
                cp_wq(g + 2).start(); cp_k(g + 2).start(); cp_v(g + 2).start(); cp_wo(g + 2).start()
            cp_wq(g + 1).wait(); cp_k(g + 1).wait(); cp_v(g + 1).wait(); cp_wo(g + 1).wait()
            for b in range(R, B):
                slot(g, b)
            for b in range(R):
                slot(g + 1, b)
            return 0
        lax.fori_loop(0, NG - 1, loop_body, 0)
        done = [t for t in osched[:R] if 0 <= t < 5]
        for b in range(R, B):
            for t in done[:2]: fin(t)
            done = done[2:]
            slot(NG - 1, b, last=True)
        O(NG - 1, 5, True)
        for t in range(6):
            cp_o(t).wait()

    out = pl.pallas_call(
        kern,
        in_specs=[pl.BlockSpec(memory_space=pl.ANY)] * 5,
        out_specs=pl.BlockSpec(memory_space=pl.ANY),
        out_shape=jax.ShapeDtypeStruct((B * SQ, D), BF),
        scratch_shapes=[
            pltpu.VMEM((B * SQ, D), BF),
            pltpu.VMEM((NG, B, KR + 32, DH), BF),
            pltpu.VMEM((NG, B, KR + 32, DH), BF),
            pltpu.VMEM((NG, D, GW), BF),
            pltpu.VMEM((NG, D, GW), BF),
            pltpu.VMEM((4, SQ, GW), BF),
            pltpu.VMEM((2, G, SQ, 128), BF),
            pltpu.VMEM((2, G, SQ, 128), F32),
            pltpu.VMEM((B * SQ, GW), BF),
            pltpu.VMEM((D, B * SQ), F32),
            pltpu.VMEM((B * SQ, D), BF),
            pltpu.SemaphoreType.DMA((5, NG)),
            pltpu.SemaphoreType.DMA((6,)),
        ],
        compiler_params=pltpu.CompilerParams(vmem_limit_bytes=100 * 1024 * 1024),
    )(x.reshape(B * SQ, D), k_cache.reshape(B, H * SK, DH), v_cache.reshape(B, H * SK, DH), wq, wo.T)
    return out.reshape(B, SQ, D)
```
